```python
import os as _os
_os.environ.setdefault("JAX_PLATFORMS", "cpu")
import jax
import jax.numpy as jnp

def _softmax(x, axis=-1):
    return jax.nn.softmax(x, axis=axis)
def _gelu(x):
    return jax.nn.gelu(x, approximate=True)
def _silu(x):
    return jax.nn.silu(x)
def _sigmoid(x):
    return jax.nn.sigmoid(x)
def _layernorm(x, axis=-1, eps=1e-5):
    m = jnp.mean(x, axis=axis, keepdims=True)
    v = jnp.var(x, axis=axis, keepdims=True)
    return (x - m) / jnp.sqrt(v + eps)
def _scatter_add(tgt, idx, src, axis=0):
    return tgt.at[idx].add(src)
def _segment_sum(src, seg, n):
    return jax.ops.segment_sum(src, seg, n)
class _Rng:
    def __init__(self, key):
        self._k = key
    def _next(self):
        self._k, sub = jax.random.split(self._k)
        return sub
    def normal(self, shape):
        return jax.random.normal(self._next(), shape, dtype=jnp.bfloat16)
    def randint(self, lo, hi, shape):
        return jax.random.randint(self._next(), shape, lo, hi, dtype=jnp.int32)
    def uniform(self, shape, lo=0.0, hi=1.0):
        return jax.random.uniform(self._next(), shape, jnp.bfloat16, lo, hi)
    def permutation(self, n):
        return jax.random.permutation(self._next(), n)


kernel_name = 'standalone__seq2seq_rnn_t_joint__speech'

def setup_inputs():
    _rng = _Rng(jax.random.key(int.from_bytes(__import__("os").urandom(4), "little")))
    _w = (lambda a: (lambda t: t.astype(jnp.bfloat16) if jnp.issubdtype(t.dtype, jnp.floating) else t)(jnp.asarray(a)))
    B, T, D, K = 2, 1000, 512, 31
    U = 8
    sc = (1.0 / (K * D)) ** 0.5
    sd = (1.0 / D) ** 0.5
    return {
        "x": _w((lambda *s: _rng.normal(s) * 0.4)(B, T, D) * 0.5),
        "w1": _w((lambda *s: _rng.normal(s) * 1.6)(K, D, D) * sc),
        "w2": _w((lambda *s: _rng.normal(s) * 1.6)(K, D, D) * sc),
        "g": _w((lambda *s: _rng.normal(s) * 1.6)(B, U, D) * 0.5),
        "w_f": _w((lambda *s: _rng.normal(s) * 1.6)(D, D) * sd),
        "w_g": _w((lambda *s: _rng.normal(s) * 1.6)(D, D) * sd),
        "w_o": _w((lambda *s: _rng.normal(s) * 1.6)(D, D) * sd),
    }

def reference(x, w1, w2, g, w_f, w_g, w_o):
    B, T, D = x.shape
    K = w1.shape[0]
    pad = K // 2
    xp = jnp.pad(x, ((0,0),(pad,pad),(0,0)))
    h = jnp.zeros_like(x)
    for i in range(K):
        h = h + jnp.einsum("btc,cd->btd", xp[:, i:i+T, :], w1[i])
    h = _gelu(h)[:, ::2, :]
    T1 = h.shape[1]
    hp = jnp.pad(h, ((0,0),(pad,pad),(0,0)))
    f = jnp.zeros_like(h)
    for i in range(K):
        f = f + jnp.einsum("btc,cd->btd", hp[:, i:i+T1, :], w2[i])
    f = _gelu(f)[:, ::2, :]
    fe = jnp.einsum("btd,de->bte", f, w_f)
    ge = jnp.einsum("bud,de->bue", g, w_g)
    j = jnp.tanh(fe[:, :, None, :] + ge[:, None, :, :])
    return jnp.einsum("btud,dv->btuv", j, w_o)
```

```python
import numpy as np
import jax
import jax.numpy as jnp
import jax.experimental.pallas as pl
import jax.experimental.pallas.tpu as pltpu

_D = 512
_L = 3
_R = 1 << _L
_J = 16 // _R
_NP = 3 ** _L
_ISSUE = {0: (1,), 1: (2, 4), 2: (3, 5), 3: (6, 7, -1)}
_F32 = jnp.float32
_BF16 = jnp.bfloat16


def _weight_sets(level):
    if level == 0:
        return [(0,)]
    h = 1 << (level - 1)
    sub = _weight_sets(level - 1)
    out = []
    for offs in ((0,), (0, h), (h,)):
        out += [tuple(sorted(o + i for o in offs for i in s)) for s in sub]
    return out


def _data_combos(z):
    if len(z) == 1:
        return [z[0]]
    h = (len(z) + 1) // 4
    n = 2 * h - 1
    z0, z1, z2 = z[0:n], z[h:h + n], z[2 * h:2 * h + n]
    return (_data_combos([a - b for a, b in zip(z0, z1)]) + _data_combos(z1)
            + _data_combos([a - b for a, b in zip(z2, z1)]))


def _out_combos(m):
    if len(m) == 1:
        return [m[0]]
    n = len(m) // 3
    m1, m2, m3 = (_out_combos(m[i * n:(i + 1) * n]) for i in range(3))
    return [a + b for a, b in zip(m1, m2)] + [a + b for a, b in zip(m2, m3)]


_WSETS = _weight_sets(_L)
_SUMS = [s for s in _WSETS if len(s) > 1]
_NS = len(_SUMS)


def _gelu(x):
    c = float(np.sqrt(2.0 / np.pi))
    return x * (0.5 * (1.0 + jnp.tanh(c * (x + 0.044715 * (x * x * x)))))


def _pack(ev, od):
    w = pltpu.pack_elementwise([ev, od], packed_dtype=_BF16)
    return w if w.dtype == jnp.uint32 else pltpu.bitcast(w, jnp.uint32)


def _unpack(w, i):
    return pltpu.unpack_elementwise(w, index=i, packed_dtype=_BF16, unpacked_dtype=_F32)


def _wsum(src, s, memo):
    if len(s) == 1:
        return src(s[0])
    if s not in memo:
        bit = _R >> 1
        while True:
            a = tuple(i for i in s if not i & bit)
            b = tuple(i for i in s if i & bit)
            if a and b:
                break
            bit >>= 1
        u, v = _wsum(src, a, memo), _wsum(src, b, memo)
        memo[s] = _pack(_unpack(u, 0) + _unpack(v, 0), _unpack(u, 1) + _unpack(v, 1))
    return memo[s]


def _kernel(x_hbm, w1_hbm, w2_hbm, g_hbm, wf_hbm, wg_hbm, wo_hbm, o_hbm,
            xb, wb, zs, dc, acc, acc2, fe, gb, sw, ob, sem_w, sem_m, sem_o):
    def w_copies(step):
        src = w1_hbm if step < 2 * _J else w2_hbm
        base = 0 if step < 2 * _J else 32
        j, e = (step % (2 * _J)) // 2, step % 2
        taps = [2 * (_R * j + r) + e for r in range(_R)]
        src = src.bitcast(jnp.uint32)
        return [pltpu.make_async_copy(src.at[t, :, pl.ds(128 * c, 128)], wb.at[base + t, c],
                                      sem_w.at[step])
                for t in taps if t < 31 for c in range(4)]

    cxs = [pltpu.make_async_copy(x_hbm.bitcast(jnp.uint32).at[:, pl.ds(128 * c, 128)],
                                 xb.at[c, pl.ds(0, 1000)], sem_m.at[0])
           for c in range(4)]
    small = [pltpu.make_async_copy(wf_hbm, sw.at[0], sem_m.at[1]),
             pltpu.make_async_copy(wg_hbm, sw.at[1], sem_m.at[2]),
             pltpu.make_async_copy(wo_hbm, sw.at[2], sem_m.at[3]),
             pltpu.make_async_copy(g_hbm, gb, sem_m.at[4])]
    for c in cxs:
        c.start()

    zero_w = jnp.zeros((4, _D // 2, 128), jnp.uint32)
    wb[31] = zero_w
    wb[63] = zero_w
    acc[...] = jnp.zeros_like(acc)
    acc2[...] = jnp.zeros_like(acc2)

    sub8 = jax.lax.broadcasted_iota(jnp.int32, (8, _D), 0)

    def from_prev_seg(v):
        return jnp.where(sub8 == 0, 0.0, pltpu.roll(v, 1, 0))

    def from_next_seg(v):
        return jnp.where(sub8 == 7, 0.0, pltpu.roll(v, 7, 0))

    def put(n, b, v):
        zs[n & 1, pl.ds((n >> 1) * 16 + 8 * b, 8), :] = v

    def make_combos(ntau):
        for e in range(2):
            for t in range(ntau):
                for cl in range(_D // 128):
                    ls = pl.ds(cl * 128, 128)
                    za, zb = ([zs[e, pl.ds((_R * t + c) * 16 + 8 * h, 8), ls]
                               for c in range(2 * _R - 1)] for h in range(2))
                    for k, (va, vb) in enumerate(zip(_data_combos(za), _data_combos(zb))):
                        dc[k, e, pl.ds(t * 8, 8), ls] = _pack(va, vb)

    for c in cxs:
        c.wait()
    for c in w_copies(0):
        c.start()
    for ip in range(64):
        for b in range(2):
            w = jnp.concatenate([xb[c, pl.ds(500 * b + ip, 8, stride=64), :] for c in range(4)],
                                axis=1)
            if ip >= 52:
                w = jnp.where(sub8 == 7, jnp.uint32(0), w)
            lo = pltpu.bitcast(w << 16, _F32)
            hi = pltpu.bitcast(w & jnp.uint32(0xFFFF0000), _F32)
            for n, v in ((2 * ip + 15, lo), (2 * ip + 16, hi)):
                put(n, b, v)
                if n - 128 >= 0:
                    put(n - 128, b, from_prev_seg(v))
                if n + 128 < 160:
                    put(n + 128, b, from_next_seg(v))
    make_combos(64 // _R + _J - 1)

    def wait_w(step):
        last = (step % (2 * _J)) == 2 * _J - 1
        for r in range(_R):
            cp = pltpu.make_async_copy(wb.at[0], wb.at[0], sem_w.at[step])
            if r < _R - 1:
                cp.wait()
            else:
                pl.when(jnp.logical_not(last))(cp.wait)

    def conv_step(step, accr, m_rows):
        j = (step % (2 * _J)) // 2
        e = step % 2
        base = (step // (2 * _J)) * 32 + 2 * _R * j + e
        wait_w(step)
        for st, todo in _ISSUE.items():
            @pl.when(step == st)
            def _():
                for t in todo:
                    for c in (small if t < 0 else w_copies(t)):
                        c.start()
        memo = [{} for _ in range(4)]
        for k, s in enumerate(_WSETS):
            rhs = jnp.concatenate(
                [_wsum(lambda r: wb[base + 2 * r, c], s, memo[c]) for c in range(4)], axis=1)
            rhs = pltpu.bitcast(rhs, _BF16)
            lhs = pltpu.bitcast(dc[k, e, pl.ds(pl.multiple_of(j * 8, 8), m_rows // 2), :], _BF16)
            accr[k] += jnp.dot(lhs, rhs, preferred_element_type=_F32)

    m1 = 16 * 64 // _R

    def body1(i, c):
        conv_step(i, acc, m1)
        return c
    jax.lax.fori_loop(jnp.int32(0), jnp.int32(2 * _J), body1, 0)

    for t in range(64 // _R):
        ys = [_out_combos([acc[k, pl.ds(t * 16 + 8 * h, 8), :] for k in range(_NP)])
              for h in range(2)]
        for rho in range(_R):
            p = _R * t + rho
            v0, v1 = _gelu(ys[0][rho]), _gelu(ys[1][rho])
            if p >= 500 - 448:
                v1 = jnp.where(sub8 >= 6, 0.0, v1)
            n = p + 15
            put(n, 0, v0)
            put(n, 1, v1)
            if n - 64 >= 0:
                r0, r1 = pltpu.roll(v0, 2, 0), pltpu.roll(v1, 2, 0)
                put(n - 64, 0, jnp.where(sub8 < 2, 0.0, r0))
                put(n - 64, 1, jnp.where(sub8 < 2, r0, r1))
            if n + 64 < 94:
                r0, r1 = pltpu.roll(v0, 6, 0), pltpu.roll(v1, 6, 0)
                put(n + 64, 0, jnp.where(sub8 >= 6, r1, r0))
                put(n + 64, 1, jnp.where(sub8 >= 6, 0.0, r1))
    make_combos(32 // _R + _J - 1)
    m2 = 16 * 32 // _R

    def body2(i, c):
        conv_step(i, acc2, m2)
        return c
    jax.lax.fori_loop(jnp.int32(2 * _J), jnp.int32(4 * _J), body2, 0)

    for c in small:
        c.wait()
    fs = []
    for t in range(32 // _R):
        ys = _out_combos([acc2[k, pl.ds(t * 16, 16), :] for k in range(_NP)])
        fs += [_gelu(y).astype(_BF16) for y in ys]
    fe[...] = jnp.dot(jnp.concatenate(fs, axis=0), sw[0], preferred_element_type=_F32)
    gl = jnp.concatenate([gb[0].astype(_F32), gb[1].astype(_F32)], axis=0).astype(_BF16)
    ge = jnp.dot(gl, sw[1], preferred_element_type=_F32)

    outs = []
    for s in range(8):
        for b in range(2):
            nq = 32 if s < 7 else 250 - 224
            geb = ge[8 * b:8 * b + 8, :]
            js = []
            for q in range(nq):
                r = 2 * s + b
                row = fe[pl.ds(q * 16 + 2 * (r % 8) + r // 8, 1), :]
                js.append(jnp.tanh(jnp.broadcast_to(row, (8, _D)) + geb))
            jv = jnp.concatenate(js, axis=0).astype(_BF16)
            o = jnp.dot(jv, sw[2], preferred_element_type=_F32).astype(_BF16)
            r0 = b * 2000 + 256 * s
            ob[pl.ds(r0, 8 * nq), :] = o
            cp = pltpu.make_async_copy(ob.at[pl.ds(r0, 8 * nq)], o_hbm.at[pl.ds(r0, 8 * nq)],
                                       sem_o.at[2 * s + b])
            cp.start()
            outs.append(cp)
    for cp in outs:
        cp.wait()


@jax.jit
def pallas_standalone__seq2seq_rnn_t_joint__speech_kernel(x, w1, w2, g, w_f, w_g, w_o):
    any_spec = pl.BlockSpec(memory_space=pl.ANY)
    out = pl.pallas_call(
        _kernel,
        out_shape=jax.ShapeDtypeStruct((4000, _D), _BF16),
        in_specs=[any_spec] * 7,
        out_specs=any_spec,
        scratch_shapes=[
            pltpu.VMEM((4, 1016, 128), jnp.uint32),
            pltpu.VMEM((64, 4, _D // 2, 128), jnp.uint32),
            pltpu.VMEM((2, 80 * 16, _D), _F32),
            pltpu.VMEM((_NP, 2, (64 // _R + _J - 1) * 8, _D), jnp.uint32),
            pltpu.VMEM((_NP, 16 * 64 // _R, _D), _F32),
            pltpu.VMEM((_NP, 16 * 32 // _R, _D), _F32),
            pltpu.VMEM((512, _D), _F32),
            pltpu.VMEM((2, 8, _D), _BF16),
            pltpu.VMEM((3, _D, _D), _BF16),
            pltpu.VMEM((4000, _D), _BF16),
            pltpu.SemaphoreType.DMA((4 * _J,)),
            pltpu.SemaphoreType.DMA((5,)),
            pltpu.SemaphoreType.DMA((16,)),
        ],
        compiler_params=pltpu.CompilerParams(vmem_limit_bytes=110 * 2 ** 20),
    )(x.reshape(2000, _D), w1, w2, g, w_f, w_g, w_o)
    return out.reshape(2, 250, 8, _D)
```

```python
import numpy as np
import jax
import jax.numpy as jnp
import jax.experimental.pallas as pl
import jax.experimental.pallas.tpu as pltpu

_D = 512
_F32 = jnp.float32
_BF16 = jnp.bfloat16


def _weight_sets(level):
    if level == 0:
        return [(0,)]
    h = 1 << (level - 1)
    sub = _weight_sets(level - 1)
    out = []
    for offs in ((0,), (0, h), (h,)):
        out += [tuple(sorted(o + i for o in offs for i in s)) for s in sub]
    return out


def _data_combos(z, emit):
    if len(z) == 1:
        emit(z[0]())
        return
    h = (len(z) + 1) // 4
    n = 2 * h - 1

    def diff(u, v):
        vals = [tuple(x - y for x, y in zip(a(), b())) for a, b in zip(u, v)]
        return [(lambda t=t: t) for t in vals]
    _data_combos(diff(z[0:n], z[h:h + n]), emit)
    _data_combos(z[h:h + n], emit)
    _data_combos(diff(z[2 * h:2 * h + n], z[h:h + n]), emit)


def _out_combos(load, lo, n):
    if n == 1:
        return [load(lo)]
    n //= 3
    m1, m2 = _out_combos(load, lo, n), _out_combos(load, lo + n, n)
    y0 = [tuple(x + y for x, y in zip(a, b)) for a, b in zip(m1, m2)]
    m3 = _out_combos(load, lo + 2 * n, n)
    return y0 + [tuple(x + y for x, y in zip(a, b)) for a, b in zip(m2, m3)]


def _halves(s):
    bit = 1 << (max(s).bit_length() - 1)
    while True:
        a = tuple(i for i in s if not i & bit)
        b = tuple(i for i in s if i & bit)
        if a and b:
            return a, b
        bit >>= 1


def _product_order(level):
    wsets = _weight_sets(level)
    sums, seen = [], set()

    def visit(s):
        if len(s) > 1 and s not in seen:
            seen.add(s)
            for h in _halves(s):
                visit(h)
            sums.append(s)
    for s in sorted(wsets, key=lambda s: (max(s), -len(s))):
        visit(s)
    raws = sorted(s for s in wsets if len(s) == 1)
    nraw, order = len(raws), []
    for i, s in enumerate(sums):
        while raws and (len(order) - i) * len(sums) <= i * nraw:
            order.append(raws.pop(0))
        order.append(s)
    return [(wsets.index(s), s) for s in order + raws]


class _Conv:
    def __init__(self, level, npos):
        self.r = 1 << level
        self.j = 16 // self.r
        self.np = 3 ** level
        self.nt = npos // self.r
        self.m = 16 * self.nt
        self.order = _product_order(level)


_C1 = _Conv(4, 64)
_C2 = _Conv(3, 32)
_GROUPS = ((0, 1), (2, 3), (4, 5, 6, 7), (8, 9, 10, 11), (12, 13, 14, 15))
_NG = len(_GROUPS)
_ISSUE = {(0, 0): [(0, 4)], (0, 24): [(1, 0), (1, 1), (1, 2)],
          (0, 42): [(1, 3), (1, 4), (2, 0)],
          (1, 0): [(2, 1)], (1, 24): [(2, 2)], (1, 42): [(2, 3)]}


def _gelu(x):
    c = float(np.sqrt(2.0 / np.pi))
    return x * (0.5 * (1.0 + jnp.tanh(c * (x + 0.044715 * (x * x * x)))))


def _pack(ev, od):
    w = pltpu.pack_elementwise([ev, od], packed_dtype=_BF16)
    return w if w.dtype == jnp.uint32 else pltpu.bitcast(w, jnp.uint32)


def _unpack(w, i):
    return pltpu.unpack_elementwise(w, index=i, packed_dtype=_BF16, unpacked_dtype=_F32)


def _wsum(src, s, memo):
    if len(s) == 1:
        return src(s[0])
    if s not in memo:
        a, b = _halves(s)
        u, v = _wsum(src, a, memo), _wsum(src, b, memo)
        if u is None or v is None:
            return v if u is None else u
        memo[s] = _pack(_unpack(u, 0) + _unpack(v, 0), _unpack(u, 1) + _unpack(v, 1))
    return memo[s]


def _kernel(x_hbm, w1_hbm, w2_hbm, g_hbm, wf_hbm, wg_hbm, wo_hbm, o_hbm,
            xb, wb, zs, dc, dc2, acc, acc2, fe, gb, sw, ob, sem_w, sem_x, sem_m, sem_o):
    w32 = (w1_hbm.bitcast(jnp.uint32), w2_hbm.bitcast(jnp.uint32))

    def w_copies(which, taps, sem):
        return [pltpu.make_async_copy(w32[which].at[t, :, pl.ds(128 * c, 128)],
                                      wb.at[32 * which + t, c], sem_w.at[sem])
                for t in taps if t < 31 for c in range(4)]

    def w1_group(e, p):
        return w_copies(0, [2 * r + e for r in _GROUPS[p]], e * _NG + p)

    def w2_group(st):
        return w_copies(1, [16 * (st // 2) + 2 * r + st % 2 for r in range(8)], 2 * _NG + st)

    cxs = [pltpu.make_async_copy(x_hbm.bitcast(jnp.uint32).at[:, pl.ds(128 * c, 128)],
                                 xb.at[c, pl.ds(0, 1000)], sem_x.at[c])
           for c in range(4)]
    small = [pltpu.make_async_copy(wf_hbm, sw.at[0], sem_m.at[1]),
             pltpu.make_async_copy(wg_hbm, sw.at[1], sem_m.at[2]),
             pltpu.make_async_copy(wo_hbm, sw.at[2], sem_m.at[3]),
             pltpu.make_async_copy(g_hbm, gb, sem_m.at[4])]
    for c in cxs:
        c.start()

    wb[31] = jnp.zeros((4, _D // 2, 128), jnp.uint32)
    wb[63] = jnp.zeros((4, _D // 2, 128), jnp.uint32)
    acc[...] = jnp.zeros_like(acc)
    acc2[...] = jnp.zeros_like(acc2)

    sub = jax.lax.broadcasted_iota(jnp.int32, (8, 128), 0)

    def put(c, n, h, v):
        zs[c, n & 1, pl.ds((n >> 1) * 16 + 8 * h, 8), :] = v

    def make_combos(cv, dst, c):
        for e in range(2):
            for t in range(cv.nt + cv.j - 1):
                cnt = iter(range(cv.np))

                def emit(v):
                    dst[next(cnt), e, c, pl.ds(t * 8, 8), :] = _pack(*v)
                _data_combos([(lambda i=i: tuple(
                    zs[c, e, pl.ds((cv.r * t + i) * 16 + 8 * h, 8), :] for h in range(2)))
                    for i in range(2 * cv.r - 1)], emit)

    def xprep(c, carry):
        pltpu.make_async_copy(xb.at[0, pl.ds(0, 1000)], xb.at[0, pl.ds(0, 1000)],
                              sem_x.at[c]).wait()
        for cv, cps in ((0, w1_group(0, 0) + w1_group(0, 1)), (1, w1_group(0, 2)), (3, w1_group(0, 3))):
            @pl.when(c == cv)
            def _():
                for cp in cps:
                    cp.start()
        for ip in range(64):
            for b in range(2):
                w = xb[c, pl.ds(500 * b + ip, 8, stride=64), :]
                if ip >= 52:
                    w = jnp.where(sub == 7, jnp.uint32(0), w)
                for n, v in ((2 * ip + 15, _unpack(w, 0)), (2 * ip + 16, _unpack(w, 1))):
                    put(c, n, b, v)
                    if n - 128 >= 0:
                        put(c, n - 128, b, jnp.where(sub == 0, 0.0, pltpu.roll(v, 1, 0)))
                    if n + 128 < 160:
                        put(c, n + 128, b, jnp.where(sub == 7, 0.0, pltpu.roll(v, 7, 0)))
        make_combos(_C1, dc, c)
        return carry
    jax.lax.fori_loop(0, 4, xprep, 0)

    def product(lhs_u32, rhs_cols):
        rhs = pltpu.bitcast(jnp.concatenate(rhs_cols, axis=1), _BF16)
        return jnp.dot(pltpu.bitcast(lhs_u32, _BF16), rhs, preferred_element_type=_F32)

    def body1(e, carry):
        memo = [{} for _ in range(4)]
        waited = set()
        for pos, (k, s) in enumerate(_C1.order):
            wait = [p for p in range(_NG) if p not in waited and set(s) & set(_GROUPS[p])]
            wait = [0, 1, 2] if pos == 0 else wait
            waited.update(wait)
            for ev in range(2):
                issue = _ISSUE.get((ev, pos), ())
                if wait or issue:
                    @pl.when(e == ev)
                    def _():
                        for p in wait:
                            for cp in w1_group(ev, p):
                                cp.wait()
                        for a, p in issue:
                            for cp in (w1_group(a, p) if a < 2 else w2_group(p)):
                                cp.start()
            cols = [_wsum(lambda r: wb[2 * r + e, c], s, memo[c]) for c in range(4)]
            lhs = jnp.concatenate([dc[k, e, c] for c in range(4)], axis=1)
            acc[k] += product(lhs, cols)
        return carry
    jax.lax.fori_loop(0, 2, body1, 0)

    def hprep(c, carry):
        ls = pl.ds(pl.multiple_of(128 * c, 128), 128)
        for t in range(_C1.nt):
            ys = _out_combos(lambda k: tuple(acc[k, pl.ds(t * 16 + 8 * h, 8), ls]
                                             for h in range(2)), 0, _C1.np)
            for rho in range(_C1.r):
                p = _C1.r * t + rho
                v0, v1 = _gelu(ys[rho][0]), _gelu(ys[rho][1])
                if p >= 500 - 448:
                    v1 = jnp.where(sub >= 6, 0.0, v1)
                n = p + 15
                put(c, n, 0, v0)
                put(c, n, 1, v1)
                if n - 64 >= 0:
                    r0, r1 = pltpu.roll(v0, 2, 0), pltpu.roll(v1, 2, 0)
                    put(c, n - 64, 0, jnp.where(sub < 2, 0.0, r0))
                    put(c, n - 64, 1, jnp.where(sub < 2, r0, r1))
                if n + 64 < 94:
                    r0, r1 = pltpu.roll(v0, 6, 0), pltpu.roll(v1, 6, 0)
                    put(c, n + 64, 0, jnp.where(sub >= 6, r1, r0))
                    put(c, n + 64, 1, jnp.where(sub >= 6, 0.0, r1))
        make_combos(_C2, dc2, c)
        return carry
    jax.lax.fori_loop(0, 4, hprep, 0)

    for cp in small:
        cp.start()

    def body2(i, carry):
        j, e = i // 2, i % 2
        base = 32 + 2 * _C2.r * j + e
        for st in range(2 * _C2.j):
            @pl.when(i == st)
            def _():
                for cp in w2_group(st):
                    cp.wait()
        memo = [{} for _ in range(4)]
        for k, s in _C2.order:
            cols = [_wsum(lambda r: wb[base + 2 * r, c], s, memo[c]) for c in range(4)]
            lhs = jnp.concatenate([dc2[k, e, c, pl.ds(pl.multiple_of(j * 8, 8), _C2.m // 2), :]
                                   for c in range(4)], axis=1)
            acc2[k] += product(lhs, cols)
        return carry
    jax.lax.fori_loop(jnp.int32(0), jnp.int32(2 * _C2.j), body2, 0)

    for c in small:
        c.wait()
    fs = []
    for t in range(_C2.nt):
        ys = _out_combos(lambda k: (acc2[k, pl.ds(t * 16, 16), :],), 0, _C2.np)
        fs += [_gelu(y[0]).astype(_BF16) for y in ys]
    fe[...] = jnp.dot(jnp.concatenate(fs, axis=0), sw[0], preferred_element_type=_F32)
    gl = jnp.concatenate([gb[0].astype(_F32), gb[1].astype(_F32)], axis=0).astype(_BF16)
    ge = jnp.dot(gl, sw[1], preferred_element_type=_F32)

    outs = []
    for s in range(8):
        for b in range(2):
            nq = 32 if s < 7 else 250 - 224
            geb = ge[8 * b:8 * b + 8, :]
            js = []
            for q in range(nq):
                r = 2 * s + b
                row = fe[pl.ds(q * 16 + 2 * (r % 8) + r // 8, 1), :]
                js.append(jnp.tanh(jnp.broadcast_to(row, (8, _D)) + geb))
            jv = jnp.concatenate(js, axis=0).astype(_BF16)
            o = jnp.dot(jv, sw[2], preferred_element_type=_F32).astype(_BF16)
            r0 = b * 2000 + 256 * s
            ob[pl.ds(r0, 8 * nq), :] = o
            cp = pltpu.make_async_copy(ob.at[pl.ds(r0, 8 * nq)], o_hbm.at[pl.ds(r0, 8 * nq)],
                                       sem_o.at[2 * s + b])
            cp.start()
            outs.append(cp)
    for cp in outs:
        cp.wait()


@jax.jit
def pallas_standalone__seq2seq_rnn_t_joint__speech_kernel(x, w1, w2, g, w_f, w_g, w_o):
    any_spec = pl.BlockSpec(memory_space=pl.ANY)
    out = pl.pallas_call(
        _kernel,
        out_shape=jax.ShapeDtypeStruct((4000, _D), _BF16),
        in_specs=[any_spec] * 7,
        out_specs=any_spec,
        scratch_shapes=[
            pltpu.VMEM((4, 1016, 128), jnp.uint32),
            pltpu.VMEM((64, 4, _D // 2, 128), jnp.uint32),
            pltpu.VMEM((4, 2, 80 * 16, 128), _F32),
            pltpu.VMEM((_C1.np, 2, 4, (_C1.nt + _C1.j - 1) * 8, 128), jnp.uint32),
            pltpu.VMEM((_C2.np, 2, 4, (_C2.nt + _C2.j - 1) * 8, 128), jnp.uint32),
            pltpu.VMEM((_C1.np, _C1.m, _D), _F32),
            pltpu.VMEM((_C2.np, _C2.m, _D), _F32),
            pltpu.VMEM((512, _D), _F32),
            pltpu.VMEM((2, 8, _D), _BF16),
            pltpu.VMEM((3, _D, _D), _BF16),
            pltpu.VMEM((4000, _D), _BF16),
            pltpu.SemaphoreType.DMA((32,)),
            pltpu.SemaphoreType.DMA((4,)),
            pltpu.SemaphoreType.DMA((5,)),
            pltpu.SemaphoreType.DMA((16,)),
        ],
        compiler_params=pltpu.CompilerParams(vmem_limit_bytes=110 * 2 ** 20),
    )(x.reshape(2000, _D), w1, w2, g, w_f, w_g, w_o)
    return out.reshape(2, 250, 8, _D)
```
